```python
import os as _os
_os.environ.setdefault("JAX_PLATFORMS", "cpu")
import jax
import jax.numpy as jnp

def _softmax(x, axis=-1):
    return jax.nn.softmax(x, axis=axis)
def _gelu(x):
    return jax.nn.gelu(x, approximate=True)
def _silu(x):
    return jax.nn.silu(x)
def _sigmoid(x):
    return jax.nn.sigmoid(x)
def _layernorm(x, axis=-1, eps=1e-5):
    m = jnp.mean(x, axis=axis, keepdims=True)
    v = jnp.var(x, axis=axis, keepdims=True)
    return (x - m) / jnp.sqrt(v + eps)
def _scatter_add(tgt, idx, src, axis=0):
    return tgt.at[idx].add(src)
def _segment_sum(src, seg, n):
    return jax.ops.segment_sum(src, seg, n)
class _Rng:
    def __init__(self, key):
        self._k = key
    def _next(self):
        self._k, sub = jax.random.split(self._k)
        return sub
    def normal(self, shape):
        return jax.random.normal(self._next(), shape, dtype=jnp.bfloat16)
    def randint(self, lo, hi, shape):
        return jax.random.randint(self._next(), shape, lo, hi, dtype=jnp.int32)
    def uniform(self, shape, lo=0.0, hi=1.0):
        return jax.random.uniform(self._next(), shape, jnp.bfloat16, lo, hi)
    def permutation(self, n):
        return jax.random.permutation(self._next(), n)


kernel_name = 'sequential_preLN__compressed_kv_cla__dense_activation_mish__decode'

def setup_inputs():
    _rng = _Rng(jax.random.key(int.from_bytes(__import__("os").urandom(4), "little")))
    _w = (lambda a: (lambda t: t.astype(jnp.bfloat16) if jnp.issubdtype(t.dtype, jnp.floating) else t)(jnp.asarray(a)))
    def _A_setup():
        B, H, Sq, Sk, D, M = 2, 32, 1, 8192, 128, 512
        Dc = 4 * D
        return {
            "x": _w((lambda *s: _rng.normal(s) * 0.05)(B, Sq, M)),
            "c_kv": _w((lambda *s: _rng.normal(s) * 0.8)(B, Sk, Dc)),
            "w_q": _w((lambda *s: _rng.normal(s) * 0.8)(M, H, D) * (M ** -0.5)),
            "w_uk": _w((lambda *s: _rng.normal(s) * 0.8)(Dc, H, D) * (Dc ** -0.5)),
            "w_uv": _w((lambda *s: _rng.normal(s) * 0.8)(Dc, H, D) * (Dc ** -0.5)),
            "w_o": _w((lambda *s: _rng.normal(s) * 0.8)(H, D, M) * ((H * D) ** -0.5)),
        }
    _A_in = _A_setup()

    def _B_setup():
        B, S, D, F = 2, 1, 512, 1792
        return {
            "x": _w((lambda *s: _rng.normal(s) * 0.05)(B, S, D)),
            "w1": _w((lambda *s: _rng.normal(s) * 0.4)(D, F) * (D ** -0.5)),
            "b1": _w((lambda *s: _rng.normal(s) * 0.05)(F)),
            "w2": _w((lambda *s: _rng.normal(s) * 0.05)(F, D) * (F ** -0.5)),
        }
    _B_in = _B_setup()

    return {
        "A_x": _A_in["x"],
        "A_c_kv": _A_in["c_kv"],
        "A_w_q": _A_in["w_q"],
        "A_w_uk": _A_in["w_uk"],
        "A_w_uv": _A_in["w_uv"],
        "A_w_o": _A_in["w_o"],
        "B_x": _B_in["x"],
        "B_w1": _B_in["w1"],
        "B_b1": _B_in["b1"],
        "B_w2": _B_in["w2"],
    }

def reference(A_x, A_c_kv, A_w_q, A_w_uk, A_w_uv, A_w_o, B_x, B_w1, B_b1, B_w2):
    def _A_ref(x, c_kv, w_q, w_uk, w_uv, w_o):
        B, Sq, M = x.shape[0], x.shape[1], x.shape[2]
        Sk = c_kv.shape[1]
        H, D = w_q.shape[1], w_q.shape[2]
        q = jnp.einsum("bqm,mhd->bhqd", x, w_q)
        k = jnp.einsum("bkc,chd->bhkd", c_kv, w_uk)
        v = jnp.einsum("bkc,chd->bhkd", c_kv, w_uv)
        scores = jnp.einsum("bhqd,bhkd->bhqk", q, k) * (D ** -0.5)
        off = Sk - Sq
        qi = jnp.arange(Sq)[:, None]
        kj = jnp.arange(Sk)[None, :]
        cmask = kj <= (qi + off)
        scores = jnp.where(cmask[None, None], scores, -1e9)
        p = _softmax(scores, axis=-1)
        ctx = jnp.einsum("bhqk,bhkd->bhqd", p, v)
        return jnp.einsum("bhqd,hdm->bqm", ctx, w_o)

    def _B_ref(x, w1, b1, w2):
        h = jnp.einsum("bsd,df->bsf", x, w1) + b1
        sp = jnp.log1p(jnp.exp(-jnp.abs(h))) + jnp.where(h > 0, h, jnp.zeros_like(h))
        act = h * jnp.tanh(sp)
        return jnp.einsum("bsf,fd->bsd", act, w2)

    x = A_x
    h = x + _A_ref(_layernorm(x, axis=-1), A_c_kv, A_w_q, A_w_uk, A_w_uv, A_w_o)
    h2 = h + _B_ref(_layernorm(h, axis=-1), B_w1, B_b1, B_w2)
    return h2
```

```python
import contextlib

import jax
import jax.numpy as jnp
from jax import lax
from jax.experimental import pallas as pl
from jax.experimental.pallas import tpu as pltpu

_SCOPES = False


def _scope(name):
    return jax.named_scope(name) if _SCOPES else contextlib.nullcontext()

F32 = jnp.float32
BF16 = jnp.bfloat16

B, H, D = 2, 32, 128
C = 512
SK = 8192
M = 512
F = 1792
EPS = 1e-5
BH = B * H

W_ROWS = 2048
N_W = (C * H) // W_ROWS
KV_T = 1024
N_KV = (B * SK) // KV_T
KV_PER_B = SK // KV_T
WO_ROWS = 512
N_WO = (H * D) // WO_ROWS
W1_ROWS = 128
N_W1 = M // W1_ROWS
W2_ROWS = 256
N_W2 = F // W2_ROWS

_counts = (N_W, N_W, N_KV, N_W, N_WO, N_W1, N_W2)
SEM_BASE = tuple(sum(_counts[:i]) for i in range(len(_counts)))
N_SEMS = sum(_counts)


def _layernorm(x):
    mu = jnp.mean(x, axis=-1, keepdims=True)
    xc = x - mu
    var = jnp.mean(xc * xc, axis=-1, keepdims=True)
    return xc * lax.rsqrt(var + EPS)


def _nt_dot(a, b):
    return lax.dot_general(a, b, (((1,), (1,)), ((), ())), preferred_element_type=F32)


def _kernel(x_ref, b1_ref, ckv_hbm, wq_hbm, wuk_hbm, wuv_hbm, wo_hbm, w1_hbm, w2_hbm,
            o_ref,
            ckv, wq, wuk, wuv, wo, w1, w2, eexp, lhs, qabs_t, ctxh, sems):

    s_wq, s_wuk, s_ckv, s_wuv, s_wo, s_w1, s_w2 = SEM_BASE

    def chunk_copy(src, dst, sem_base, j, rows):
        off = j * rows
        if not isinstance(j, int):
            off = pl.multiple_of(off, rows)
        return pltpu.make_async_copy(src.at[pl.ds(off, rows)], dst.at[pl.ds(off, rows)],
                                     sems.at[sem_base + j])

    with _scope('issue'):
        for src, dst, sem, n, rows in (
                (wq_hbm, wq, s_wq, N_W, W_ROWS),
                (wuk_hbm, wuk, s_wuk, N_W, W_ROWS),
                (ckv_hbm, ckv, s_ckv, N_KV, KV_T),
                (wuv_hbm, wuv, s_wuv, N_W, W_ROWS),
                (wo_hbm, wo, s_wo, N_WO, WO_ROWS),
                (w1_hbm, w1, s_w1, N_W1, W1_ROWS),
                (w2_hbm, w2, s_w2, N_W2, W2_ROWS)):
            for j in range(n):
                chunk_copy(src, dst, sem, j, rows).start()

    with _scope('consts'):
        e_r = lax.broadcasted_iota(jnp.int32, (128, 32 * 128), 0)
        e_l = lax.broadcasted_iota(jnp.int32, (128, 32 * 128), 1)
        eexp[...] = jnp.where((e_l // H) == e_r, 1.0, 0.0).astype(BF16)

        bd_n = lax.broadcasted_iota(jnp.int32, (BH, 32 * 128), 0)
        bd_k = lax.broadcasted_iota(jnp.int32, (BH, 32 * 128), 1)
        bd_mask = (bd_k % H) == (bd_n % H)

        def build_lhs(src):
            for i in range(4):
                rep = jnp.dot(src[:, 128 * i:128 * (i + 1)], eexp[...], preferred_element_type=F32)
                lhs[:, 4096 * i:4096 * (i + 1)] = jnp.where(bd_mask, rep, 0.0).astype(BF16)

        def blockdiag_matmul(w_hbm, w_vmem, sem):
            def body(j, acc):
                chunk_copy(w_hbm, w_vmem, sem, j, W_ROWS).wait()
                off = pl.multiple_of(j * W_ROWS, W_ROWS)
                return acc + jnp.dot(lhs[:, pl.ds(off, W_ROWS)], w_vmem[pl.ds(off, W_ROWS), :],
                                     preferred_element_type=F32)
            return lax.fori_loop(0, N_W, body, jnp.zeros((BH, D), F32))

    with _scope('q'):
        x = x_ref[...].astype(F32)
        xn = _layernorm(x).astype(BF16).astype(F32)
        row64 = lax.broadcasted_iota(jnp.int32, (BH, M), 0)
        xsrc = jnp.where(row64 < H, xn[0:1, :], xn[1:2, :]).astype(BF16)
        build_lhs(xsrc)
        q = blockdiag_matmul(wq_hbm, wq, s_wq).astype(BF16)

    with _scope('qabs'):
        m_h = lax.broadcasted_iota(jnp.int32, (H, BH), 0)
        m_n = lax.broadcasted_iota(jnp.int32, (H, BH), 1)
        head_mask = (m_n % H) == m_h
        x_per_chunk = W_ROWS // H

        def qabs_body(j, carry):
            chunk_copy(wuk_hbm, wuk, s_wuk, j, W_ROWS).wait()
            off = pl.multiple_of(j * W_ROWS, W_ROWS)
            r = _nt_dot(wuk[pl.ds(off, W_ROWS), :], q)
            r3 = r.reshape(x_per_chunk, H, BH)
            red = jnp.sum(jnp.where(head_mask[None], r3, 0.0), axis=1)
            qabs_t[pl.ds(pl.multiple_of(j * x_per_chunk, x_per_chunk), x_per_chunk), :] = red
            return carry
        lax.fori_loop(0, N_W, qabs_body, 0)
        qa = (qabs_t[...] * (D ** -0.5)).T.astype(BF16)

    with _scope('attn'):
        ctx_parts = []
        for b in range(B):
            qa_b = qa[b * H:(b + 1) * H, :]

            def attn_body(i, carry, b=b, qa_b=qa_b):
                m_prev, l_prev, acc = carry
                j = b * KV_PER_B + i
                chunk_copy(ckv_hbm, ckv, s_ckv, j, KV_T).wait()
                cc = ckv[pl.ds(pl.multiple_of(j * KV_T, KV_T), KV_T), :]
                s = _nt_dot(qa_b, cc)
                m_new = jnp.maximum(m_prev, jnp.max(s, axis=-1, keepdims=True))
                alpha = jnp.exp(m_prev - m_new)
                p = jnp.exp(s - m_new)
                l_new = alpha * l_prev + jnp.sum(p, axis=-1, keepdims=True)
                acc = alpha * acc + jnp.dot(p.astype(BF16), cc, preferred_element_type=F32)
                return m_new, l_new, acc

            m0 = jnp.full((H, 1), -jnp.inf, F32)
            l0 = jnp.zeros((H, 1), F32)
            a0 = jnp.zeros((H, C), F32)
            _, l_f, acc_f = lax.fori_loop(0, KV_PER_B, attn_body, (m0, l0, a0))
            ctx_parts.append(acc_f / l_f)
        ctx_c = jnp.concatenate(ctx_parts, axis=0).astype(BF16)

    with _scope('ctx'):
        build_lhs(ctx_c)
        ctx = blockdiag_matmul(wuv_hbm, wuv, s_wuv).astype(BF16)

    with _scope('oproj'):
        s_r = lax.broadcasted_iota(jnp.int32, (8 * H, BH), 0)
        s_n = lax.broadcasted_iota(jnp.int32, (8 * H, BH), 1)
        sel = jnp.where(s_n == (s_r // 8) + H * (s_r % 8), 1.0, 0.0).astype(BF16)
        ctxh[...] = jnp.dot(sel, ctx, preferred_element_type=F32)

        heads_per_chunk = WO_ROWS // D

        def oproj_body(j, acc):
            chunk_copy(wo_hbm, wo, s_wo, j, WO_ROWS).wait()
            for hh in range(heads_per_chunk):
                h = j * heads_per_chunk + hh
                lh = ctxh[pl.ds(pl.multiple_of(8 * h, 8), 8), :].astype(BF16)
                acc = acc + jnp.dot(lh, wo[pl.ds(pl.multiple_of(D * h, D), D), :],
                                    preferred_element_type=F32)
            return acc
        attn = lax.fori_loop(0, N_WO, oproj_body, jnp.zeros((8, M), F32))

    with _scope('ffn'):
        h1 = x + attn[0:B, :]
        hn = _layernorm(h1).astype(BF16)

        hid = jnp.zeros((B, F), F32)
        for k in range(N_W1):
            chunk_copy(w1_hbm, w1, s_w1, k, W1_ROWS).wait()
            hid = hid + jnp.dot(hn[:, W1_ROWS * k:W1_ROWS * (k + 1)], w1[W1_ROWS * k:W1_ROWS * (k + 1), :],
                                preferred_element_type=F32)
        b1 = jnp.concatenate([b1_ref[r:r + 1, :] for r in range(F // 128)], axis=1).astype(F32)
        hid = hid + b1
        sp = jnp.log1p(jnp.exp(-jnp.abs(hid))) + jnp.maximum(hid, 0.0)
        act = (hid * jnp.tanh(sp)).astype(BF16)

        out = h1
        for k in range(N_W2):
            chunk_copy(w2_hbm, w2, s_w2, k, W2_ROWS).wait()
            out = out + jnp.dot(act[:, W2_ROWS * k:W2_ROWS * (k + 1)], w2[W2_ROWS * k:W2_ROWS * (k + 1), :],
                                preferred_element_type=F32)
        o_ref[...] = out.astype(o_ref.dtype)


@jax.jit
def pallas_sequential_preLN__compressed_kv_cla__dense_activation_mish__decode_kernel(
    A_x: jax.Array,
    A_c_kv: jax.Array,
    A_w_q: jax.Array,
    A_w_uk: jax.Array,
    A_w_uv: jax.Array,
    A_w_o: jax.Array,
    B_x: jax.Array,
    B_w1: jax.Array,
    B_b1: jax.Array,
    B_w2: jax.Array,
):
    del B_x
    x2 = A_x.reshape(B, M)
    ckv2 = A_c_kv.reshape(B * SK, C)
    wq2 = A_w_q.reshape(M * H, D)
    wuk2 = A_w_uk.reshape(C * H, D)
    wuv2 = A_w_uv.reshape(C * H, D)
    wo2 = A_w_o.reshape(H * D, M)
    b12 = B_b1.reshape(F // 128, 128)

    vmem = pl.BlockSpec(memory_space=pltpu.VMEM)
    hbm = pl.BlockSpec(memory_space=pl.ANY)
    dma = pltpu.SemaphoreType.DMA
    out = pl.pallas_call(
        _kernel,
        out_shape=jax.ShapeDtypeStruct((B, M), jnp.bfloat16),
        in_specs=[vmem, vmem, hbm, hbm, hbm, hbm, hbm, hbm, hbm],
        out_specs=vmem,
        scratch_shapes=[
            pltpu.VMEM((B * SK, C), BF16),
            pltpu.VMEM((M * H, D), BF16),
            pltpu.VMEM((C * H, D), BF16),
            pltpu.VMEM((C * H, D), BF16),
            pltpu.VMEM((H * D, M), BF16),
            pltpu.VMEM((M, F), BF16),
            pltpu.VMEM((F, M), BF16),
            pltpu.VMEM((128, 32 * 128), BF16),
            pltpu.VMEM((BH, C * H), BF16),
            pltpu.VMEM((C, BH), F32),
            pltpu.VMEM((8 * H, D), F32),
            dma((N_SEMS,)),
        ],
        compiler_params=pltpu.CompilerParams(vmem_limit_bytes=100 * 1024 * 1024),
    )(x2, b12, ckv2, wq2, wuk2, wuv2, wo2, B_w1, B_w2)
    return out.reshape(B, 1, M)
```

```python
import jax
import jax.numpy as jnp
from jax import lax
from jax.experimental import pallas as pl
from jax.experimental.pallas import tpu as pltpu

F32 = jnp.float32
BF16 = jnp.bfloat16

B, H, D = 2, 32, 128
C = 512
SK = 8192
M = 512
F = 1792
EPS = 1e-5
BH = B * H

W_ROWS = 2048
N_W = (C * H) // W_ROWS
KV_T = 1024
N_KV = (B * SK) // KV_T
KV_PER_B = SK // KV_T
WO_ROWS = 512
N_WO = (H * D) // WO_ROWS
W1_ROWS = 128
N_W1 = M // W1_ROWS
W2_SIZES = (256, 256, 256, 256, 256, 256, 128, 128)
W2_OFFS = tuple(sum(W2_SIZES[:i]) for i in range(len(W2_SIZES)))
N_W2 = len(W2_SIZES)
assert sum(W2_SIZES) == F

_counts = (1, 1, N_W, N_W, N_KV, N_W, N_WO, N_W1, N_W2)
SEM_BASE = tuple(sum(_counts[:i]) for i in range(len(_counts)))
N_SEMS = sum(_counts)


def _layernorm(x):
    mu = jnp.mean(x, axis=-1, keepdims=True)
    xc = x - mu
    var = jnp.mean(xc * xc, axis=-1, keepdims=True)
    return xc * lax.rsqrt(var + EPS)


def _nt_dot(a, b):
    return lax.dot_general(a, b, (((1,), (1,)), ((), ())), preferred_element_type=F32)


def _kernel(*refs):
    pl.run_scoped(lambda sems: _body(*refs, sems), pltpu.SemaphoreType.DMA((N_SEMS,)))


def _body(x_hbm, b1_hbm, ckv_hbm, wq_hbm, wuk_hbm, wuv_hbm, wo_hbm, w1_hbm, w2_hbm,
          o_ref,
          x_ref, b1_ref, ckv, wq, wuk, wuv, wo, w1, w2, eexp, lhs, qabs_t, ctxh, sems):
    s_x, s_b1, s_wq, s_wuk, s_ckv, s_wuv, s_wo, s_w1, s_w2 = SEM_BASE

    def chunk_copy(src, dst, sem_base, j, rows):
        off = j * rows
        if not isinstance(j, int):
            off = pl.multiple_of(off, rows)
        return pltpu.make_async_copy(src.at[pl.ds(off, rows)], dst.at[pl.ds(off, rows)],
                                     sems.at[sem_base + j])

    def w2_copy(k):
        return pltpu.make_async_copy(w2_hbm.at[pl.ds(W2_OFFS[k], W2_SIZES[k])],
                                     w2.at[pl.ds(W2_OFFS[k], W2_SIZES[k])], sems.at[s_w2 + k])

    for src, dst, sem, n, rows in (
            (x_hbm, x_ref, s_x, 1, B),
            (b1_hbm, b1_ref, s_b1, 1, F // 128),
            (wq_hbm, wq, s_wq, N_W, W_ROWS),
            (wuk_hbm, wuk, s_wuk, N_W, W_ROWS),
            (ckv_hbm, ckv, s_ckv, N_KV, KV_T),
            (wuv_hbm, wuv, s_wuv, N_W, W_ROWS),
            (wo_hbm, wo, s_wo, N_WO, WO_ROWS),
            (w1_hbm, w1, s_w1, N_W1, W1_ROWS)):
        for j in range(n):
            chunk_copy(src, dst, sem, j, rows).start()
    for k in range(N_W2):
        w2_copy(k).start()

    e_r = lax.broadcasted_iota(jnp.int32, (128, H * 128), 0)
    e_l = lax.broadcasted_iota(jnp.int32, (128, H * 128), 1)
    eexp[...] = jnp.where((e_l // H) == e_r, 1.0, 0.0).astype(BF16)

    bd_n = lax.broadcasted_iota(jnp.int32, (BH, H * 128), 0)
    bd_k = lax.broadcasted_iota(jnp.int32, (BH, H * 128), 1)
    bd_mask = (bd_k % H) == (bd_n % H)

    def build_lhs(src):
        for i in range(4):
            rep = jnp.dot(src[:, 128 * i:128 * (i + 1)], eexp[...], preferred_element_type=F32)
            lhs[:, H * 128 * i:H * 128 * (i + 1)] = jnp.where(bd_mask, rep, 0.0).astype(BF16)

    def blockdiag_matmul(w_hbm, w_vmem, sem):
        def body(j, acc):
            chunk_copy(w_hbm, w_vmem, sem, j, W_ROWS).wait()
            off = pl.multiple_of(j * W_ROWS, W_ROWS)
            return acc + jnp.dot(lhs[:, pl.ds(off, W_ROWS)], w_vmem[pl.ds(off, W_ROWS), :],
                                 preferred_element_type=F32)
        return lax.fori_loop(0, N_W, body, jnp.zeros((BH, D), F32))

    chunk_copy(x_hbm, x_ref, s_x, 0, B).wait()
    x = x_ref[...].astype(F32)
    xn = _layernorm(x).astype(BF16).astype(F32)
    row64 = lax.broadcasted_iota(jnp.int32, (BH, M), 0)
    xsrc = jnp.where(row64 < H, xn[0:1, :], xn[1:2, :]).astype(BF16)
    build_lhs(xsrc)
    q = blockdiag_matmul(wq_hbm, wq, s_wq).astype(BF16)

    m_h = lax.broadcasted_iota(jnp.int32, (H, BH), 0)
    m_n = lax.broadcasted_iota(jnp.int32, (H, BH), 1)
    head_mask = (m_n % H) == m_h
    x_per_chunk = W_ROWS // H

    def qabs_body(j, carry):
        chunk_copy(wuk_hbm, wuk, s_wuk, j, W_ROWS).wait()
        off = pl.multiple_of(j * W_ROWS, W_ROWS)
        r = _nt_dot(wuk[pl.ds(off, W_ROWS), :], q)
        r3 = r.reshape(x_per_chunk, H, BH)
        red = jnp.sum(jnp.where(head_mask[None], r3, 0.0), axis=1)
        qabs_t[pl.ds(pl.multiple_of(j * x_per_chunk, x_per_chunk), x_per_chunk), :] = red
        return carry
    lax.fori_loop(0, N_W, qabs_body, 0)
    qa = (qabs_t[...] * (D ** -0.5)).T.astype(BF16)

    ctx_parts = []
    for b in range(B):
        qa_b = qa[b * H:(b + 1) * H, :]

        def attn_body(i, carry, b=b, qa_b=qa_b):
            m_prev, l_prev, acc = carry
            j = b * KV_PER_B + i
            chunk_copy(ckv_hbm, ckv, s_ckv, j, KV_T).wait()
            cc = ckv[pl.ds(pl.multiple_of(j * KV_T, KV_T), KV_T), :]
            s = _nt_dot(qa_b, cc)
            m_new = jnp.maximum(m_prev, jnp.max(s, axis=-1, keepdims=True))
            alpha = jnp.exp(m_prev - m_new)
            p = jnp.exp(s - m_new)
            l_new = alpha * l_prev + jnp.sum(p, axis=-1, keepdims=True)
            acc = alpha * acc + jnp.dot(p.astype(BF16), cc, preferred_element_type=F32)
            return m_new, l_new, acc

        m0 = jnp.full((H, 1), -jnp.inf, F32)
        l0 = jnp.zeros((H, 1), F32)
        a0 = jnp.zeros((H, C), F32)
        _, l_f, acc_f = lax.fori_loop(0, KV_PER_B, attn_body, (m0, l0, a0))
        ctx_parts.append(acc_f / l_f)
    ctx_c = jnp.concatenate(ctx_parts, axis=0).astype(BF16)

    build_lhs(ctx_c)
    ctx = blockdiag_matmul(wuv_hbm, wuv, s_wuv).astype(BF16)

    s_r = lax.broadcasted_iota(jnp.int32, (8 * H, BH), 0)
    s_n = lax.broadcasted_iota(jnp.int32, (8 * H, BH), 1)
    sel = jnp.where(s_n == (s_r // 8) + H * (s_r % 8), 1.0, 0.0).astype(BF16)
    ctxh[...] = jnp.dot(sel, ctx, preferred_element_type=F32)

    heads_per_chunk = WO_ROWS // D

    def oproj_body(j, acc):
        chunk_copy(wo_hbm, wo, s_wo, j, WO_ROWS).wait()
        for hh in range(heads_per_chunk):
            h = j * heads_per_chunk + hh
            lh = ctxh[pl.ds(pl.multiple_of(8 * h, 8), 8), :].astype(BF16)
            acc = acc + jnp.dot(lh, wo[pl.ds(pl.multiple_of(D * h, D), D), :],
                                preferred_element_type=F32)
        return acc
    attn = lax.fori_loop(0, N_WO, oproj_body, jnp.zeros((8, M), F32))

    h1 = x + attn[0:B, :]
    hn = _layernorm(h1).astype(BF16)

    hid = jnp.zeros((B, F), F32)
    for k in range(N_W1):
        chunk_copy(w1_hbm, w1, s_w1, k, W1_ROWS).wait()
        hid = hid + jnp.dot(hn[:, W1_ROWS * k:W1_ROWS * (k + 1)],
                            w1[W1_ROWS * k:W1_ROWS * (k + 1), :], preferred_element_type=F32)
    chunk_copy(b1_hbm, b1_ref, s_b1, 0, F // 128).wait()
    b1 = jnp.concatenate([b1_ref[r:r + 1, :] for r in range(F // 128)], axis=1).astype(F32)
    hid = hid + b1
    sp = jnp.log1p(jnp.exp(-jnp.abs(hid))) + jnp.maximum(hid, 0.0)
    act = (hid * jnp.tanh(sp)).astype(BF16)

    out = h1
    for k in range(N_W2):
        w2_copy(k).wait()
        o, n = W2_OFFS[k], W2_SIZES[k]
        out = out + jnp.dot(act[:, o:o + n], w2[o:o + n, :], preferred_element_type=F32)
    o_ref[...] = out.astype(o_ref.dtype)


@jax.jit
def pallas_sequential_preLN__compressed_kv_cla__dense_activation_mish__decode_kernel(
    A_x: jax.Array,
    A_c_kv: jax.Array,
    A_w_q: jax.Array,
    A_w_uk: jax.Array,
    A_w_uv: jax.Array,
    A_w_o: jax.Array,
    B_x: jax.Array,
    B_w1: jax.Array,
    B_b1: jax.Array,
    B_w2: jax.Array,
):
    del B_x
    assert A_x.shape == (B, 1, M) and A_c_kv.shape == (B, SK, C)
    assert A_w_q.shape == (M, H, D) and A_w_uk.shape == (C, H, D) and A_w_uv.shape == (C, H, D)
    assert A_w_o.shape == (H, D, M) and B_w1.shape == (M, F) and B_w2.shape == (F, M)
    assert B_b1.shape == (F,)

    x2 = A_x.reshape(B, M)
    ckv2 = A_c_kv.reshape(B * SK, C)
    wq2 = A_w_q.reshape(M * H, D)
    wuk2 = A_w_uk.reshape(C * H, D)
    wuv2 = A_w_uv.reshape(C * H, D)
    wo2 = A_w_o.reshape(H * D, M)
    b12 = B_b1.reshape(F // 128, 128)

    hbm = pl.BlockSpec(memory_space=pl.ANY)
    out = pl.pallas_call(
        _kernel,
        out_shape=jax.ShapeDtypeStruct((B, M), jnp.bfloat16),
        in_specs=[hbm] * 9,
        out_specs=pl.BlockSpec(memory_space=pltpu.VMEM),
        scratch_shapes=[
            pltpu.VMEM((B, M), BF16),
            pltpu.VMEM((F // 128, 128), BF16),
            pltpu.VMEM((B * SK, C), BF16),
            pltpu.VMEM((M * H, D), BF16),
            pltpu.VMEM((C * H, D), BF16),
            pltpu.VMEM((C * H, D), BF16),
            pltpu.VMEM((H * D, M), BF16),
            pltpu.VMEM((M, F), BF16),
            pltpu.VMEM((F, M), BF16),
            pltpu.VMEM((128, H * 128), BF16),
            pltpu.VMEM((BH, C * H), BF16),
            pltpu.VMEM((C, BH), F32),
            pltpu.VMEM((8 * H, D), F32),
        ],
        compiler_params=pltpu.CompilerParams(vmem_limit_bytes=64 * 1024 * 1024),
    )(x2, b12, ckv2, wq2, wuk2, wuv2, wo2, B_w1, B_w2)
    return out.reshape(B, 1, M)
```
